```python
import jax
import jax.numpy as jnp

def _softmax(x, axis=-1):
    return jax.nn.softmax(x, axis=axis)
def _gelu(x):
    return jax.nn.gelu(x, approximate=True)
def _silu(x):
    return jax.nn.silu(x)
def _sigmoid(x):
    return jax.nn.sigmoid(x)
def _layernorm(x, axis=-1, eps=1e-5):
    m = jnp.mean(x, axis=axis, keepdims=True)
    v = jnp.var(x, axis=axis, keepdims=True)
    return (x - m) / jnp.sqrt(v + eps)
def _scatter_add(tgt, idx, src, axis=0):
    return tgt.at[idx].add(src)
def _segment_sum(src, seg, n):
    return jax.ops.segment_sum(src, seg, n)
class _Rng:
    def __init__(self, key):
        self._k = key
    def _next(self):
        self._k, sub = jax.random.split(self._k)
        return sub
    def normal(self, shape):
        return jax.random.normal(self._next(), shape, dtype=jnp.bfloat16)
    def randint(self, lo, hi, shape):
        return jax.random.randint(self._next(), shape, lo, hi, dtype=jnp.int32)
    def uniform(self, shape, lo=0.0, hi=1.0):
        return jax.random.uniform(self._next(), shape, jnp.bfloat16, lo, hi)
    def permutation(self, n):
        return jax.random.permutation(self._next(), n)


kernel_name = 'standalone__instancenorm__prompt'

def setup_inputs():
    _rng = _Rng(jax.random.key(int.from_bytes(__import__("os").urandom(4), "little")))
    _w = (lambda a: (lambda t: t.astype(jnp.bfloat16) if jnp.issubdtype(t.dtype, jnp.floating) else t)(jnp.asarray(a)))
    B, C, H, W = 2, 1024, 2048, 32
    return {
        "x": _w((lambda *s: _rng.normal(s) * 0.05)(B, C, H, W)),
        "g": _w((lambda *s: _rng.normal(s) * 0.05)(C) + 1.0),
        "b": _w((lambda *s: _rng.normal(s) * 0.05)(C)),
    }

def reference(x, g, b):
    mu = x.mean(axis=(-2, -1), keepdims=True)
    var = ((x - mu) * (x - mu)).mean(axis=(-2, -1), keepdims=True)
    xhat = (x - mu) / jnp.sqrt(var + 1e-5)
    return xhat * g.reshape(1, -1, 1, 1) + b.reshape(1, -1, 1, 1)
```

```python
import jax
import jax.numpy as jnp
import jax.experimental.pallas as pl
import jax.experimental.pallas.tpu as pltpu

EPS = 1e-5
CHUNK = 16
NCHUNK = 44
UNROLL = 4
RWIN = 8


def _make(chunk, nchunk, unroll, S, ws, opt):
    def kernel(g_in, b_in, x_hbm, o_hbm, buf, acc, mu_t, rs_t, gv, bv_, g_ref, b_ref, sem, psem):
        n_inst, W, H = x_hbm.shape
        C = g_ref.shape[0]
        per_round = chunk * nchunk
        n_rounds = -(-n_inst // per_round)
        tot = n_inst // chunk
        inv_n = 1.0 / (W * H)
        nt = H // 128

        def tile(k, i):
            return buf[k, :, pl.ds(i * 128, 128)].astype(jnp.float32)

        def fold(a):
            p = [a[r:r + 8] for r in range(0, W, 8)]
            while len(p) > 1:
                p = [p[r] + p[r + 1] for r in range(0, len(p), 2)]
            return p[0]

        def loop(fn):
            def body(i, _):
                for u in range(unroll):
                    fn(i * unroll + u)
            jax.lax.fori_loop(0, chunk // unroll, body, None)

        def finish():
            s = acc[pl.ds(0, chunk, stride=8), :]
            for r in range(1, 8):
                s = s + acc[pl.ds(r, chunk, stride=8), :]
            s = jnp.sum(s, axis=1, keepdims=True) * inv_n
            return jnp.broadcast_to(s, (chunk, 128))

        PR = 8
        ppi = W // PR
        npc = chunk * ppi
        WS, WM = ws

        def start(r, j, write):
            if 'nodma' in opt:
                return
            if write:
                L = npc // WS
                ipg = L // ppi
                i0 = (j // WM) * (WM * chunk) + (j % WM) * ipg
                stride = WM * ipg
                ns = WS
            else:
                L = npc // S
                i0 = j * chunk
                stride = L // ppi
                ns = S
            for t in range(npc):
                st, k = t % ns, t // ns
                i = i0 + (st * stride + k // ppi)
                rows = pl.ds((k % ppi) * PR, PR)
                h = (o_hbm if write else x_hbm).at[r * per_round + i, rows]
                v = buf.at[i, rows]
                src, dst = (v, h) if write else (h, v)
                pltpu.make_async_copy(src, dst, sem.at[int(write), j % 2]).start(priority=t % 2)

        def wait(j, write):
            if 'nodma' in opt:
                return
            v = buf.at[pl.ds(j * chunk, chunk)]
            pltpu.make_async_copy(v, v, sem.at[int(write), j % 2]).wait()

        def compute(r, j):
            base = j * chunk

            def pa(i):
                a = tile(base + i, 0)
                for t in range(1, nt):
                    a = a + tile(base + i, t)
                acc[pl.ds(pl.multiple_of(i * 8, 8), 8), :] = fold(a)
            loop(pa)
            mu_t[...] = finish()

            def pb(i):
                mu = mu_t[pl.ds(i, 1), :]
                a = None
                for t in range(nt):
                    d = tile(base + i, t) - mu
                    d = d * d
                    a = d if a is None else a + d
                acc[pl.ds(pl.multiple_of(i * 8, 8), 8), :] = fold(a)
            loop(pb)
            rs_t[...] = jax.lax.rsqrt(finish() + EPS)

            def pc(i):
                c = (r * per_round + base + i) % C
                mu = mu_t[pl.ds(i, 1), :]
                a = rs_t[pl.ds(i, 1), :] * g_ref[c]
                bv = b_ref[c]
                for t in range(nt):
                    y = (tile(base + i, t) - mu) * a + bv
                    buf[base + i, :, pl.ds(t * 128, 128)] = y.astype(buf.dtype)
            loop(pc)

        E = 3 if 'V' in opt else 2
        start(0, 0, False)
        start(0, 1, False)
        gv[...] = g_in[...].astype(jnp.float32)
        bv_[...] = b_in[...].astype(jnp.float32)
        cg = pltpu.make_async_copy(gv, g_ref, psem.at[0])
        cb = pltpu.make_async_copy(bv_, b_ref, psem.at[1])
        cg.start()
        cb.start()
        cg.wait()
        cb.wait()

        def round_(r, _):
            nch = jnp.minimum(nchunk, tot - r * nchunk)

            @pl.when(r > 0)
            def _():
                start(r, 0, False)
                start(r, 1, False)

            def rbody(j, _):
                wait(j, False)

                @pl.when(j + 2 < nch)
                def _():
                    start(r, j + 2, False)

                @pl.when(j == nch - E)
                def _():
                    start(r, 0, True)

                @pl.when(j == nch - 1)
                def _():
                    start(r, 1, True)
                compute(r, j)
            jax.lax.fori_loop(0, nch, rbody, None)

            def wbody(j, _):
                wait(j, True)

                @pl.when(j + 2 < nch)
                def _():
                    start(r, j + 2, True)
            jax.lax.fori_loop(0, nch, wbody, None)

        jax.lax.fori_loop(0, n_rounds, round_, None)
    return kernel


def _build(chunk=CHUNK, nchunk=NCHUNK, unroll=UNROLL, S=RWIN, ws=(16,4), opt=''):
    def f(x, g, b):
        B, C, H, W = x.shape
        xt = x.transpose(0, 1, 3, 2).reshape(B * C, W, H)
        o = pl.pallas_call(
            _make(chunk, nchunk, unroll, S, ws, opt),
            in_specs=[pl.BlockSpec(), pl.BlockSpec(),
                      pl.BlockSpec(memory_space=pl.ANY)],
            out_specs=pl.BlockSpec(memory_space=pl.ANY),
            out_shape=jax.ShapeDtypeStruct(xt.shape, xt.dtype),
            scratch_shapes=[pltpu.VMEM((chunk * nchunk, W, H), x.dtype),
 pltpu.VMEM((chunk*8,128), jnp.float32), pltpu.VMEM((chunk,128), jnp.float32), pltpu.VMEM((chunk,128), jnp.float32),
                            pltpu.VMEM((C,), jnp.float32), pltpu.VMEM((C,), jnp.float32), pltpu.SMEM((C,), jnp.float32), pltpu.SMEM((C,), jnp.float32),
 pltpu.SemaphoreType.DMA((2, 2)), pltpu.SemaphoreType.DMA((2,))],
            compiler_params=pltpu.CompilerParams(vmem_limit_bytes=120 * 2**20, disable_bounds_checks=True),
        )(g, b, xt)
        return o.reshape(B, C, W, H).transpose(0, 1, 3, 2)
    return f


@jax.jit
def pallas_standalone__instancenorm__prompt_kernel(x, g, b):
    return _build()(x, g, b)
```

```python
import jax
import jax.numpy as jnp
import jax.experimental.pallas as pl
import jax.experimental.pallas.tpu as pltpu

EPS = 1e-5
CHUNK = 16
NCHUNK = 44
UNROLL = 4
PIECE_ROWS = 8
READ_STREAMS = 8
WRITE_STREAMS = 16
WRITE_SPAN = 4
LANES, SUBLANES = 128, 8


def _kernel(g_in, b_in, x_hbm, o_hbm,
            buf, acc, mu_t, rstd_t, g_f32, b_f32, g_smem, b_smem, sem, param_sem):
    n_inst, W, H = x_hbm.shape
    C = g_smem.shape[0]
    per_round = CHUNK * NCHUNK
    n_chunks = n_inst // CHUNK
    n_rounds = pl.cdiv(n_chunks, NCHUNK)
    inv_n = 1.0 / (W * H)
    n_tiles = H // LANES
    pieces_per_inst = W // PIECE_ROWS
    n_pieces = CHUNK * pieces_per_inst

    def start(r, j, write):
        if write:
            streams = WRITE_STREAMS
            inst_per_stream = CHUNK // streams
            stride = WRITE_SPAN * inst_per_stream
            first = (j // WRITE_SPAN) * (WRITE_SPAN * CHUNK) + (j % WRITE_SPAN) * inst_per_stream
        else:
            streams = READ_STREAMS
            stride = CHUNK // streams
            first = j * CHUNK
        for t in range(n_pieces):
            stream, k = t % streams, t // streams
            i = first + (stream * stride + k // pieces_per_inst)
            rows = pl.ds((k % pieces_per_inst) * PIECE_ROWS, PIECE_ROWS)
            hbm = (o_hbm if write else x_hbm).at[r * per_round + i, rows]
            vmem = buf.at[i, rows]
            src, dst = (vmem, hbm) if write else (hbm, vmem)
            pltpu.make_async_copy(src, dst, sem.at[int(write), j % 2]).start(priority=t % 2)

    def wait(j, write):
        whole = buf.at[pl.ds(j * CHUNK, CHUNK)]
        pltpu.make_async_copy(whole, whole, sem.at[int(write), j % 2]).wait()

    def tile(k, t):
        return buf[k, :, pl.ds(t * LANES, LANES)].astype(jnp.float32)

    def store_partial(i, a):
        parts = [a[s:s + SUBLANES] for s in range(0, W, SUBLANES)]
        while len(parts) > 1:
            parts = [parts[s] + parts[s + 1] for s in range(0, len(parts), 2)]
        acc[pl.ds(pl.multiple_of(i * SUBLANES, SUBLANES), SUBLANES), :] = parts[0]

    def means():
        s = acc[pl.ds(0, CHUNK, stride=SUBLANES), :]
        for sub in range(1, SUBLANES):
            s = s + acc[pl.ds(sub, CHUNK, stride=SUBLANES), :]
        s = jnp.sum(s, axis=1, keepdims=True) * inv_n
        return jnp.broadcast_to(s, (CHUNK, LANES))

    def for_instances(fn):
        @pl.loop(0, CHUNK // UNROLL)
        def _(it):
            for u in range(UNROLL):
                fn(it * UNROLL + u)

    def normalize(r, j):
        base = j * CHUNK

        @for_instances
        def _(i):
            a = tile(base + i, 0)
            for t in range(1, n_tiles):
                a = a + tile(base + i, t)
            store_partial(i, a)

        mu_t[...] = means()

        @for_instances
        def _(i):
            mu = mu_t[pl.ds(i, 1), :]
            a = None
            for t in range(n_tiles):
                d = tile(base + i, t) - mu
                a = d * d if a is None else a + d * d
            store_partial(i, a)

        rstd_t[...] = jax.lax.rsqrt(means() + EPS)

        @for_instances
        def _(i):
            c = (r * per_round + base + i) % C
            mu = mu_t[pl.ds(i, 1), :]
            scale = rstd_t[pl.ds(i, 1), :] * g_smem[c]
            shift = b_smem[c]
            for t in range(n_tiles):
                y = (tile(base + i, t) - mu) * scale + shift
                buf[base + i, :, pl.ds(t * LANES, LANES)] = y.astype(buf.dtype)

    start(0, 0, False)
    start(0, 1, False)

    g_f32[...] = g_in[...].astype(jnp.float32)
    b_f32[...] = b_in[...].astype(jnp.float32)
    g_copy = pltpu.make_async_copy(g_f32, g_smem, param_sem.at[0])
    b_copy = pltpu.make_async_copy(b_f32, b_smem, param_sem.at[1])
    g_copy.start()
    b_copy.start()
    g_copy.wait()
    b_copy.wait()

    @pl.loop(0, n_rounds)
    def _(r):
        n = jnp.minimum(NCHUNK, n_chunks - r * NCHUNK)

        @pl.when(r > 0)
        def _():
            start(r, 0, False)
            start(r, 1, False)

        @pl.loop(0, n)
        def _(j):
            wait(j, False)

            @pl.when(j + 2 < n)
            def _():
                start(r, j + 2, False)

            @pl.when(j == n - 2)
            def _():
                start(r, 0, True)

            @pl.when(j == n - 1)
            def _():
                start(r, 1, True)

            normalize(r, j)

        @pl.loop(0, n)
        def _(j):
            wait(j, True)

            @pl.when(j + 2 < n)
            def _():
                start(r, j + 2, True)


@jax.jit
def pallas_standalone__instancenorm__prompt_kernel(x, g, b):
    B, C, H, W = x.shape
    n_chunks = B * C // CHUNK
    last_round = n_chunks - (pl.cdiv(n_chunks, NCHUNK) - 1) * NCHUNK
    assert B * C % CHUNK == 0 and H % LANES == 0 and W % PIECE_ROWS == 0
    assert NCHUNK % WRITE_SPAN == 0 and last_round % WRITE_SPAN == 0
    assert last_round - 2 >= WRITE_SPAN

    xt = x.transpose(0, 1, 3, 2).reshape(B * C, W, H)
    out = pl.pallas_call(
        _kernel,
        in_specs=[pl.BlockSpec(), pl.BlockSpec(), pl.BlockSpec(memory_space=pl.ANY)],
        out_specs=pl.BlockSpec(memory_space=pl.ANY),
        out_shape=jax.ShapeDtypeStruct(xt.shape, xt.dtype),
        scratch_shapes=[
            pltpu.VMEM((CHUNK * NCHUNK, W, H), x.dtype),
            pltpu.VMEM((CHUNK * SUBLANES, LANES), jnp.float32),
            pltpu.VMEM((CHUNK, LANES), jnp.float32),
            pltpu.VMEM((CHUNK, LANES), jnp.float32),
            pltpu.VMEM((C,), jnp.float32),
            pltpu.VMEM((C,), jnp.float32),
            pltpu.SMEM((C,), jnp.float32),
            pltpu.SMEM((C,), jnp.float32),
            pltpu.SemaphoreType.DMA((2, 2)),
            pltpu.SemaphoreType.DMA((2,)),
        ],
        compiler_params=pltpu.CompilerParams(
            vmem_limit_bytes=120 * 2**20, disable_bounds_checks=True),
    )(g, b, xt)
    return out.reshape(B, C, W, H).transpose(0, 1, 3, 2)
```

```python
import jax
import jax.numpy as jnp
import jax.experimental.pallas as pl
import jax.experimental.pallas.tpu as pltpu

EPS = 1e-5
CHUNK = 16
NCHUNK = 44
UNROLL = 4
PIECE_ROWS = 8
STREAMS = 16
SPAN = 4
LAG = SPAN - 1
LANES, SUBLANES = 128, 8


def _kernel(g_in, b_in, x_hbm, o_hbm,
            buf, acc, mu_t, rstd_t, g_f32, b_f32, g_smem, b_smem, sem, param_sem):
    n_inst, W, H = x_hbm.shape
    C = g_smem.shape[0]
    per_round = CHUNK * NCHUNK
    n_chunks = n_inst // CHUNK
    n_rounds = pl.cdiv(n_chunks, NCHUNK)
    inv_n = 1.0 / (W * H)
    n_tiles = H // LANES
    pieces_per_inst = W // PIECE_ROWS
    n_pieces = CHUNK * pieces_per_inst

    def start(r, j, write):
        inst_per_stream = CHUNK // STREAMS
        stride = SPAN * inst_per_stream
        first = (j // SPAN) * (SPAN * CHUNK) + (j % SPAN) * inst_per_stream
        for t in range(n_pieces):
            stream, k = t % STREAMS, t // STREAMS
            i = first + (stream * stride + k // pieces_per_inst)
            rows = pl.ds((k % pieces_per_inst) * PIECE_ROWS, PIECE_ROWS)
            hbm = (o_hbm if write else x_hbm).at[r * per_round + i, rows]
            vmem = buf.at[i, rows]
            src, dst = (vmem, hbm) if write else (hbm, vmem)
            pltpu.make_async_copy(src, dst, sem.at[int(write), j % 2]).start(priority=t % 2)

    def wait(j, write):
        whole = buf.at[pl.ds(j * CHUNK, CHUNK)]
        pltpu.make_async_copy(whole, whole, sem.at[int(write), j % 2]).wait()

    def tile(k, t):
        return buf[k, :, pl.ds(t * LANES, LANES)].astype(jnp.float32)

    def store_partial(i, a):
        parts = [a[s:s + SUBLANES] for s in range(0, W, SUBLANES)]
        while len(parts) > 1:
            parts = [parts[s] + parts[s + 1] for s in range(0, len(parts), 2)]
        acc[pl.ds(pl.multiple_of(i * SUBLANES, SUBLANES), SUBLANES), :] = parts[0]

    def means():
        s = acc[pl.ds(0, CHUNK, stride=SUBLANES), :]
        for sub in range(1, SUBLANES):
            s = s + acc[pl.ds(sub, CHUNK, stride=SUBLANES), :]
        s = jnp.sum(s, axis=1, keepdims=True) * inv_n
        return jnp.broadcast_to(s, (CHUNK, LANES))

    def for_instances(fn):
        @pl.loop(0, CHUNK // UNROLL)
        def _(it):
            for u in range(UNROLL):
                fn(it * UNROLL + u)

    def normalize(r, j):
        base = j * CHUNK

        @for_instances
        def _(i):
            a = tile(base + i, 0)
            for t in range(1, n_tiles):
                a = a + tile(base + i, t)
            store_partial(i, a)

        mu_t[...] = means()

        @for_instances
        def _(i):
            mu = mu_t[pl.ds(i, 1), :]
            a = None
            for t in range(n_tiles):
                d = tile(base + i, t) - mu
                a = d * d if a is None else a + d * d
            store_partial(i, a)

        rstd_t[...] = jax.lax.rsqrt(means() + EPS)

        @for_instances
        def _(i):
            c = (r * per_round + base + i) % C
            mu = mu_t[pl.ds(i, 1), :]
            scale = rstd_t[pl.ds(i, 1), :] * g_smem[c]
            shift = b_smem[c]
            for t in range(n_tiles):
                y = (tile(base + i, t) - mu) * scale + shift
                buf[base + i, :, pl.ds(t * LANES, LANES)] = y.astype(buf.dtype)

    start(0, 0, False)
    start(0, 1, False)

    g_f32[...] = g_in[...].astype(jnp.float32)
    b_f32[...] = b_in[...].astype(jnp.float32)
    g_copy = pltpu.make_async_copy(g_f32, g_smem, param_sem.at[0])
    b_copy = pltpu.make_async_copy(b_f32, b_smem, param_sem.at[1])
    g_copy.start()
    b_copy.start()
    g_copy.wait()
    b_copy.wait()

    @pl.loop(0, n_rounds)
    def _(r):
        n = jnp.minimum(NCHUNK, n_chunks - r * NCHUNK)

        @pl.when(r > 0)
        def _():
            start(r, 0, False)
            start(r, 1, False)

        @pl.loop(0, n)
        def _(j):
            wait(j, False)

            @pl.when(j + 2 < n)
            def _():
                start(r, j + 2, False)

            @pl.when(j == n - 2)
            def _():
                start(r, 0, True)

            @pl.when(j == n - 1)
            def _():
                start(r, 1, True)

            @pl.when(j >= LAG)
            def _():
                normalize(r, j - LAG)

        @pl.loop(0, n)
        def _(j):
            wait(j, True)

            @pl.when(j + 2 < n)
            def _():
                start(r, j + 2, True)

            @pl.when(j < LAG)
            def _():
                normalize(r, n - LAG + j)


@jax.jit
def pallas_standalone__instancenorm__prompt_kernel(x, g, b):
    B, C, H, W = x.shape
    n_chunks = B * C // CHUNK
    last_round = n_chunks - (pl.cdiv(n_chunks, NCHUNK) - 1) * NCHUNK
    assert B * C % CHUNK == 0 and H % LANES == 0 and W % PIECE_ROWS == 0
    assert NCHUNK % SPAN == 0 and last_round % SPAN == 0 and last_round >= 3 * SPAN

    xt = x.transpose(0, 1, 3, 2).reshape(B * C, W, H)
    out = pl.pallas_call(
        _kernel,
        in_specs=[pl.BlockSpec(), pl.BlockSpec(), pl.BlockSpec(memory_space=pl.ANY)],
        out_specs=pl.BlockSpec(memory_space=pl.ANY),
        out_shape=jax.ShapeDtypeStruct(xt.shape, xt.dtype),
        scratch_shapes=[
            pltpu.VMEM((CHUNK * NCHUNK, W, H), x.dtype),
            pltpu.VMEM((CHUNK * SUBLANES, LANES), jnp.float32),
            pltpu.VMEM((CHUNK, LANES), jnp.float32),
            pltpu.VMEM((CHUNK, LANES), jnp.float32),
            pltpu.VMEM((C,), jnp.float32),
            pltpu.VMEM((C,), jnp.float32),
            pltpu.SMEM((C,), jnp.float32),
            pltpu.SMEM((C,), jnp.float32),
            pltpu.SemaphoreType.DMA((2, 2)),
            pltpu.SemaphoreType.DMA((2,)),
        ],
        compiler_params=pltpu.CompilerParams(
            vmem_limit_bytes=120 * 2**20, disable_bounds_checks=True),
    )(g, b, xt)
    return out.reshape(B, C, W, H).transpose(0, 1, 3, 2)
```
